```python
import jax
import jax.numpy as jnp

def _softmax(x, axis=-1):
    return jax.nn.softmax(x, axis=axis)
def _gelu(x):
    return jax.nn.gelu(x, approximate=True)
def _silu(x):
    return jax.nn.silu(x)
def _sigmoid(x):
    return jax.nn.sigmoid(x)
def _layernorm(x, axis=-1, eps=1e-5):
    m = jnp.mean(x, axis=axis, keepdims=True)
    v = jnp.var(x, axis=axis, keepdims=True)
    return (x - m) / jnp.sqrt(v + eps)
def _scatter_add(tgt, idx, src, axis=0):
    return tgt.at[idx].add(src)
def _segment_sum(src, seg, n):
    return jax.ops.segment_sum(src, seg, n)
class _Rng:
    def __init__(self, key):
        self._k = key
    def _next(self):
        self._k, sub = jax.random.split(self._k)
        return sub
    def normal(self, shape):
        return jax.random.normal(self._next(), shape, dtype=jnp.bfloat16)
    def randint(self, lo, hi, shape):
        return jax.random.randint(self._next(), shape, lo, hi, dtype=jnp.int32)
    def uniform(self, shape, lo=0.0, hi=1.0):
        return jax.random.uniform(self._next(), shape, jnp.bfloat16, lo, hi)
    def permutation(self, n):
        return jax.random.permutation(self._next(), n)


kernel_name = 'recurrent_scan__sliding_block_cached__dense_activation_gelu__decode'

def setup_inputs():
    _rng = _Rng(jax.random.key(int.from_bytes(__import__("os").urandom(4), "little")))
    _w = (lambda a: (lambda t: t.astype(jnp.bfloat16) if jnp.issubdtype(t.dtype, jnp.floating) else t)(jnp.asarray(a)))
    def _A_setup():
        B, Sq, D = 2, 1, 576
        Hq, Hkv, Sk, Dh = 32, 16, 32768, 128
        assert Hq % Hkv == 0, (Hq, Hkv)
        return {
            "x": _w((lambda *s: _rng.normal(s) * 0.05)(B, Sq, D)),
            "k_cache": _w((lambda *s: _rng.normal(s) * 0.05)(B, Hkv, Sk, Dh)),
            "v_cache": _w((lambda *s: _rng.normal(s) * 0.05)(B, Hkv, Sk, Dh)),
            "wq": _w((lambda *s: _rng.normal(s) * 0.05)(D, Hq * Dh) * (D ** -0.5)),
            "wo": _w((lambda *s: _rng.normal(s) * 0.05)(Hq * Dh, D) * ((Hq * Dh) ** -0.5)),
        }
    _A_in = _A_setup()

    def _B_setup():
        B, S, D, F = 2, 1, 576, 4608
        return {
            "x": _w((lambda *s: _rng.normal(s) * 0.05)(B, S, D)),
            "w1": _w((lambda *s: _rng.normal(s) * 0.05)(D, F) * (D ** -0.5)),
            "b1": _w((lambda *s: _rng.normal(s) * 0.05)(F) * 0.01),
            "w2": _w((lambda *s: _rng.normal(s) * 0.05)(F, D) * (F ** -0.5)),
            "b2": _w((lambda *s: _rng.normal(s) * 0.05)(D) * 0.01),
        }
    _B_in = _B_setup()

    return {
        "A_x": _A_in["x"],
        "A_k_cache": _A_in["k_cache"],
        "A_v_cache": _A_in["v_cache"],
        "A_wq": _A_in["wq"],
        "A_wo": _A_in["wo"],
        "B_x": _B_in["x"],
        "B_w1": _B_in["w1"],
        "B_b1": _B_in["b1"],
        "B_w2": _B_in["w2"],
        "B_b2": _B_in["b2"],
    }

def reference(A_x, A_k_cache, A_v_cache, A_wq, A_wo, B_x, B_w1, B_b1, B_w2, B_b2):
    def _A_ref(x, k_cache, v_cache, wq, wo):
        B, Sq, D = x.shape
        Hq, Dh = 32, 128
        Hkv, Sk = k_cache.shape[1], k_cache.shape[2]
        W = min(4096, max(256, Sk // 4))
        rep = Hq // Hkv
        q = (lambda x, *d: x.transpose(*d))((x @ wq).reshape(B, Sq, Hq, Dh), 0, 2, 1, 3)
        k = jnp.repeat(k_cache[:, :, Sk - W:, :], rep, axis=1)
        v = jnp.repeat(v_cache[:, :, Sk - W:, :], rep, axis=1)
        scores = jnp.einsum("bhqd,bhkd->bhqk", q, k) * (Dh ** -0.5)
        p = _softmax(scores, axis=-1)
        o = jnp.einsum("bhqk,bhkd->bhqd", p, v)
        return (lambda x, *d: x.transpose(*d))(o, 0, 2, 1, 3).reshape(B, Sq, Hq * Dh) @ wo

    def _B_ref(x, w1, b1, w2, b2):
        h = jnp.einsum("bsd,df->bsf", x, w1) + b1
        h = _gelu(h)
        return jnp.einsum("bsf,fd->bsd", h, w2) + b2

    x = A_x
    xn = _layernorm(x, axis=-1)
    s = _A_ref(xn, A_k_cache, A_v_cache, A_wq, A_wo)
    g = _silu(_B_ref(xn, B_w1, B_b1, B_w2, B_b2))
    return x + s * g
```

```python
import functools

import jax
import jax.numpy as jnp
import jax.experimental.pallas as pl
import jax.experimental.pallas.tpu as pltpu

_HQ = 32
_DH = 128
_EPS = 1e-5
_NT = (((1,), (1,)), ((), ()))
DEPTH = 2
LAST = 16


def _gelu_tanh(x):
    c = 0.7978845608028654
    return 0.5 * x * (1.0 + jnp.tanh(c * (x + 0.044715 * (x * x * x))))


def _kernel(x_hbm, k_hbm, v_hbm, wq_hbm, wot_hbm, w1_hbm, b1_hbm, w2t_hbm, b2_hbm,
            o_ref,
            x_buf, b1_buf, b2_buf, wq_buf, wot_buf, w1_buf, w2t_buf, k_buf, v_buf,
            q_buf, o_buf, xn_buf, h_buf, g_buf, sem_w, sem_k, sem_v,
            *, B, D, F, HKV, SK, W):
    s0 = SK - W
    npair = B * HKV

    def first(i):
        src, dst = [(wq_hbm, wq_buf), (x_hbm, x_buf), (b1_hbm, b1_buf), (b2_hbm, b2_buf)][i]
        return pltpu.make_async_copy(src, dst, sem_w.at[0])

    def w1copy():
        return pltpu.make_async_copy(w1_hbm, w1_buf, sem_w.at[0])

    def w2copy():
        return pltpu.make_async_copy(w2t_hbm, w2t_buf, sem_w.at[0])

    def kcopy(p):
        return pltpu.make_async_copy(
            k_hbm.at[p % B, p // B, pl.ds(s0, W), :], k_buf.at[p], sem_k.at[p % DEPTH])

    def vcopy(p):
        return pltpu.make_async_copy(
            v_hbm.at[p % B, p // B, pl.ds(s0, W), :], v_buf.at[p], sem_v.at[p % DEPTH])

    chunks = [(0, 128), (128, 128), (256, 128), (384, 128), (512 + LAST, 64 - LAST), (512, LAST)]
    csems = [sem_k.at[0], sem_v.at[0], sem_k.at[1], sem_v.at[1], sem_k.at[0], sem_v.at[0]]

    def ocopy(c):
        r0, n = chunks[c]
        return pltpu.make_async_copy(
            wot_hbm.at[pl.ds(r0, n), :], wot_buf.at[pl.ds(r0, n), :], csems[c])

    for i in range(4):
        first(i).start()

    def prime(p, c):
        kcopy(p).start()
        vcopy(p).start()
        return c

    jax.lax.fori_loop(0, DEPTH, prime, 0)

    for i in range(4):
        first(i).wait()
    x = x_buf[...].astype(jnp.float32)
    mu = jnp.mean(x, axis=-1, keepdims=True)
    xc = x - mu
    var = jnp.mean(xc * xc, axis=-1, keepdims=True)
    xn = xc * jax.lax.rsqrt(var + _EPS)
    row_d = jax.lax.broadcasted_iota(jnp.int32, (8, D), 0)
    xn8 = jnp.where(row_d % 2 == 0, xn[0:1, :], xn[1:2, :]).astype(jnp.bfloat16)
    xn_buf[...] = xn8

    q8 = jnp.dot(xn8, wq_buf[...], preferred_element_type=jnp.float32)
    q_buf[...] = q8 * (_DH ** -0.5)

    row = jax.lax.broadcasted_iota(jnp.int32, (8, _DH), 0)

    def body(p, c):
        j = p // B
        b = p % B
        off_a = pl.multiple_of(2 * j * _DH, _DH)
        off_b = pl.multiple_of((2 * j + 1) * _DH, _DH)
        qa = q_buf[:, pl.ds(off_a, _DH)]
        qb = q_buf[:, pl.ds(off_b, _DH)]
        lhs = jnp.where(row < 2, qa, qb).astype(jnp.bfloat16)
        kcopy(p).wait()

        @pl.when(p + DEPTH < npair)
        def _():
            kcopy(p + DEPTH).start()

        @pl.when(p == npair - 2)
        def _():
            ocopy(0).start()

        @pl.when(p == npair - 1)
        def _():
            ocopy(2).start()

        s = jax.lax.dot_general(lhs, k_buf[p], _NT, preferred_element_type=jnp.float32)
        m = jnp.max(s, axis=-1, keepdims=True)
        e = jnp.exp(s - m)
        l = jnp.sum(e, axis=-1, keepdims=True)
        vcopy(p).wait()

        @pl.when(p + DEPTH < npair)
        def _():
            vcopy(p + DEPTH).start()

        @pl.when(p == npair - 2)
        def _():
            ocopy(1).start()

        @pl.when(p == npair - 1)
        def _():
            ocopy(3).start()

        o = jnp.dot(e.astype(jnp.bfloat16), v_buf[p], preferred_element_type=jnp.float32)
        o = o / l
        o_sh = pltpu.roll(o, 6, 0)

        @pl.when(b == 0)
        def _():
            o_buf[:, pl.ds(off_a, _DH)] = jnp.where(row == 0, o, 0.0)
            o_buf[:, pl.ds(off_b, _DH)] = jnp.where(row == 0, o_sh, 0.0)

        @pl.when(b == 1)
        def _():
            o_buf[:, pl.ds(off_a, _DH)] = jnp.where(row == 1, o, o_buf[:, pl.ds(off_a, _DH)])
            o_buf[:, pl.ds(off_b, _DH)] = jnp.where(row == 1, o_sh, o_buf[:, pl.ds(off_b, _DH)])

        @pl.when(p == 2)
        def _():
            w1copy().start()

        @pl.when(p == 8)
        def _():
            w1copy().wait()
            w2copy().start()
            h = jnp.dot(xn_buf[...], w1_buf[...], preferred_element_type=jnp.float32)
            h = _gelu_tanh(h + b1_buf[...].astype(jnp.float32).reshape(1, F))
            h_buf[...] = h.astype(jnp.bfloat16)

        @pl.when(p == 14)
        def _():
            w2copy().wait()
            y = jax.lax.dot_general(h_buf[...], w2t_buf[...], _NT,
                                    preferred_element_type=jnp.float32)
            y = y + b2_buf[...].astype(jnp.float32).reshape(1, D)
            g_buf[...] = y * jax.nn.sigmoid(y)

        return c

    jax.lax.fori_loop(0, npair, body, 0)

    o2 = o_buf[...].astype(jnp.bfloat16)
    xf = x_buf[...].astype(jnp.float32)
    for c in range(len(chunks)):
        r0, n = chunks[c]
        ocopy(c).wait()
        if c + 4 < len(chunks):
            ocopy(c + 4).start()
        s = jax.lax.dot_general(o2, wot_buf[r0:r0 + n, :], _NT,
                                preferred_element_type=jnp.float32)
        o_ref[:, r0:r0 + n] = (xf[:, r0:r0 + n]
                               + s[0:2, :] * g_buf[0:2, r0:r0 + n]).astype(o_ref.dtype)


@jax.jit
def pallas_recurrent_scan__sliding_block_cached__dense_activation_gelu__decode_kernel(
    A_x, A_k_cache, A_v_cache, A_wq, A_wo, B_x, B_w1, B_b1, B_w2, B_b2,
):
    B, SQ, D = A_x.shape
    _, HKV, SK, DH = A_k_cache.shape
    F = B_w1.shape[1]
    W = min(4096, max(256, SK // 4))
    assert B == 2 and SQ == 1 and DH == _DH and A_wq.shape[1] == _HQ * _DH
    assert _HQ == 2 * HKV and D == 576
    bf = jnp.bfloat16
    npair = B * HKV

    any_spec = pl.BlockSpec(memory_space=pl.ANY)
    out = pl.pallas_call(
        functools.partial(_kernel, B=B, D=D, F=F, HKV=HKV, SK=SK, W=W),
        out_shape=jax.ShapeDtypeStruct((B, D), A_x.dtype),
        in_specs=[any_spec] * 9,
        out_specs=pl.BlockSpec(memory_space=pltpu.VMEM),
        scratch_shapes=[
            pltpu.VMEM((B, D), bf),
            pltpu.VMEM((F,), bf),
            pltpu.VMEM((D,), bf),
            pltpu.VMEM((D, _HQ * _DH), bf),
            pltpu.VMEM((D, _HQ * _DH), bf),
            pltpu.VMEM((D, F), bf),
            pltpu.VMEM((D, F), bf),
            pltpu.VMEM((npair, W, _DH), bf),
            pltpu.VMEM((npair, W, _DH), bf),
            pltpu.VMEM((8, _HQ * _DH), jnp.float32),
            pltpu.VMEM((8, _HQ * _DH), jnp.float32),
            pltpu.VMEM((8, D), bf),
            pltpu.VMEM((8, F), bf),
            pltpu.VMEM((8, D), jnp.float32),
            pltpu.SemaphoreType.DMA((1,)),
            pltpu.SemaphoreType.DMA((DEPTH,)),
            pltpu.SemaphoreType.DMA((DEPTH,)),
        ],
        compiler_params=pltpu.CompilerParams(vmem_limit_bytes=110 * 1024 * 1024),
    )(
        A_x.reshape(B, D), A_k_cache, A_v_cache, A_wq, A_wo.T, B_w1,
        B_b1, B_w2.T, B_b2,
    )
    return out.reshape(B, SQ, D)
```

```python
import functools

import jax
import jax.numpy as jnp
import jax.experimental.pallas as pl
import jax.experimental.pallas.tpu as pltpu

_HQ = 32
_DH = 128
_EPS = 1e-5
_NT = (((1,), (1,)), ((), ()))
_NN = (((1,), (0,)), ((), ()))

_NSLOT = 3
_PROWS = 8
_NPIECE = 37
_W1_AT = 4
_W2_AT = 10
_ROW_SPLIT = (384, 448, 512)
_TAIL_COLS = (2048, 2048)


def _dot(a, b, dims):
    return jax.lax.dot_general(a, b, dims, precision=jax.lax.Precision.DEFAULT,
                               preferred_element_type=jnp.float32)


def _gelu_tanh(x):
    c = 0.7978845608028654
    return 0.5 * x * (1.0 + jnp.tanh(c * (x + 0.044715 * (x * x * x))))


def _wo_chunks(rows, cols):
    chunks = []
    r = _NPIECE * _PROWS
    for e in _ROW_SPLIT:
        chunks.append((r, e - r, 0, cols))
        r = e
    c = 0
    for n in _TAIL_COLS:
        chunks.append((r, rows - r, c, n))
        c += n
    assert c == cols
    return chunks


def _body(x_hbm, k_hbm, v_hbm, wq_hbm, wot_hbm, w1_hbm, b1_hbm, w2t_hbm, b2_hbm, o_hbm,
          x_buf, b1_buf, b2_buf, wq_buf, wot_buf, w1_buf, w2t_buf, k_buf, v_buf,
          q_buf, o_buf, xn_buf, h_buf, g_buf, out_buf, stage,
          sem_first, sem_w, sem_k, sem_v, sem_in, sem_out, sem_c, sem_o,
          *, B, D, F, HKV, SK, W):
    s0 = SK - W
    npair = B * HKV
    HD = _HQ * _DH
    half = D // 2
    NP = _NPIECE
    A1, A2 = _W1_AT, _W2_AT
    side_rows = NP * _PROWS
    chunks = _wo_chunks(D, HD)
    assert NP <= 2 + npair + 4 - 1

    def first(i):
        src, dst = [(wq_hbm.at[pl.ds(0, half)], wq_buf.at[pl.ds(0, half)]),
                    (wq_hbm.at[pl.ds(half, half)], wq_buf.at[pl.ds(half, half)]),
                    (x_hbm, x_buf), (b1_hbm, b1_buf), (b2_hbm, b2_buf)][i]
        return pltpu.make_async_copy(src, dst, sem_first.at[i])

    def wcopy(which, h):
        src, dst = [(w1_hbm, w1_buf), (w2t_hbm, w2t_buf)][which]
        return pltpu.make_async_copy(src.at[pl.ds(h * half, half)],
                                     dst.at[pl.ds(h * half, half)], sem_w.at[h])

    def kcopy(p):
        return pltpu.make_async_copy(
            k_hbm.at[p % B, p // B, pl.ds(s0, W), :], k_buf.at[p], sem_k.at[p % 2])

    def vcopy(p):
        return pltpu.make_async_copy(
            v_hbm.at[p % B, p // B, pl.ds(s0, W), :], v_buf.at[p], sem_v.at[p % 2])

    def ocopy(c):
        r0, nr, c0, nc = chunks[c]
        return pltpu.make_async_copy(
            wot_hbm.at[pl.ds(r0, nr), pl.ds(c0, nc)],
            wot_buf.at[pl.ds(r0, nr), pl.ds(c0, nc)], sem_c.at[c])

    def rows(k):
        if isinstance(k, int):
            return pl.ds(k * _PROWS, _PROWS)
        return pl.ds(pl.multiple_of(k * _PROWS, _PROWS), _PROWS)

    def cin(k):
        return pltpu.make_async_copy(wot_hbm.at[rows(k)], stage.at[k % _NSLOT],
                                     sem_in.at[k % 2])

    def cout(k):
        return pltpu.make_async_copy(stage.at[k % _NSLOT], wot_buf.at[rows(k)],
                                     sem_out.at[0])

    def when(cond):
        if isinstance(cond, bool):
            return (lambda f: f()) if cond else (lambda f: None)
        return pl.when(cond)

    def pinned(cond, fn):
        if isinstance(cond, bool):
            when(cond)(fn)
            return

        def step(i, c):
            fn()
            return c
        jax.lax.fori_loop(0, cond.astype(jnp.int32), step, 0)

    def service(t):
        @when(t < NP)
        def _():
            cin(t).wait()

        if not (isinstance(t, int) and t == 0):
            @when(t <= NP)
            def _():
                cout(t - 1).wait()

        def starts():
            @when(t + 2 < NP)
            def _():
                cin(t + 2).start()
            cout(t).start()

        pinned(t < NP, starts)

    for i in range(5):
        first(i).start()
    cin(0).start()
    cin(1).start()

    def prime(p, c):
        kcopy(p).start()
        vcopy(p).start()
        return c

    jax.lax.fori_loop(0, 2, prime, 0)

    first(0).wait()
    service(0)
    for i in range(1, 5):
        first(i).wait()
    service(1)

    x = x_buf[...].astype(jnp.float32)
    mu = jnp.mean(x, axis=-1, keepdims=True)
    xc = x - mu
    var = jnp.mean(xc * xc, axis=-1, keepdims=True)
    xn = xc * jax.lax.rsqrt(var + _EPS)
    row_d = jax.lax.broadcasted_iota(jnp.int32, (8, D), 0)
    xn8 = jnp.where(row_d % 2 == 0, xn[0:1, :], xn[1:2, :]).astype(jnp.bfloat16)
    xn_buf[...] = xn8
    q_buf[...] = _dot(xn8, wq_buf[...], _NN)

    row = jax.lax.broadcasted_iota(jnp.int32, (8, _DH), 0)
    scale = _DH ** -0.5

    def step(p, c):
        j = p // B
        b = p % B
        off_a = pl.multiple_of(2 * j * _DH, _DH)
        off_b = pl.multiple_of((2 * j + 1) * _DH, _DH)
        tick = (2 + p + (p > A1).astype(jnp.int32) + (p > A1 + 1).astype(jnp.int32)
                + (p > A2).astype(jnp.int32) + (p > A2 + 1).astype(jnp.int32))
        lhs = jnp.where(row < 2, q_buf[:, pl.ds(off_a, _DH)],
                        q_buf[:, pl.ds(off_b, _DH)]).astype(jnp.bfloat16)
        kcopy(p).wait()
        vcopy(p).wait()

        @pl.when(p + 2 < npair)
        def _():
            kcopy(p + 2).start()
            vcopy(p + 2).start()

        @pl.when(p == npair - 2)
        def _():
            ocopy(0).start()
            ocopy(1).start()

        service(tick)

        @pl.when(p == npair - 1)
        def _():
            for c in range(2, len(chunks)):
                ocopy(c).start()

        s = _dot(lhs, k_buf[p], _NT)
        m = jnp.max(s, axis=-1, keepdims=True)
        e = jnp.exp((s - m) * scale)
        l = jnp.sum(e, axis=-1, keepdims=True)
        o = _dot(e.astype(jnp.bfloat16), v_buf[p], _NN) / l
        o_sh = pltpu.roll(o, 6, 0)

        @pl.when(b == 0)
        def _():
            o_buf[:, pl.ds(off_a, _DH)] = jnp.where(row == 0, o, 0.0)
            o_buf[:, pl.ds(off_b, _DH)] = jnp.where(row == 0, o_sh, 0.0)

        @pl.when(b == 1)
        def _():
            o_buf[:, pl.ds(off_a, _DH)] = jnp.where(row == 1, o, o_buf[:, pl.ds(off_a, _DH)])
            o_buf[:, pl.ds(off_b, _DH)] = jnp.where(row == 1, o_sh, o_buf[:, pl.ds(off_b, _DH)])

        for which, at in ((0, A1), (1, A2)):
            for h in range(2):
                @pl.when(p == at - 2 + h)
                def _():
                    wcopy(which, h).start()

        @pl.when(p == A1)
        def _():
            wcopy(0, 0).wait()
            service(2 + A1 + 1)

        @pl.when(p == A1 + 1)
        def _():
            wcopy(0, 1).wait()
            service(2 + A1 + 3)
            h = _dot(xn_buf[...], w1_buf[...], _NN)
            h = _gelu_tanh(h + b1_buf[...].astype(jnp.float32).reshape(1, F))
            h_buf[...] = h.astype(jnp.bfloat16)

        @pl.when(p == A2)
        def _():
            wcopy(1, 0).wait()
            service(2 + A2 + 3)

        @pl.when(p == A2 + 1)
        def _():
            wcopy(1, 1).wait()
            service(2 + A2 + 5)
            y = _dot(h_buf[...], w2t_buf[...], _NT)
            y = y + b2_buf[...].astype(jnp.float32).reshape(1, D)
            g_buf[...] = y * jax.nn.sigmoid(y)

        return c

    jax.lax.fori_loop(0, npair, step, 0)

    o2 = o_buf[...].astype(jnp.bfloat16)
    xf = x_buf[...].astype(jnp.float32)

    def finish(s, r0, nr):
        out_buf[:, r0:r0 + nr] = (xf[:, r0:r0 + nr]
                                  + s[0:2, :] * g_buf[0:2, r0:r0 + nr]).astype(out_buf.dtype)

    def proj(r0, r1):
        finish(_dot(o2, wot_buf[r0:r1, :], _NT), r0, r1 - r0)

    done = 0
    while done + 128 <= side_rows:
        proj(done, done + 128)
        done += 128
    acc = None
    for c, (r0, nr, c0, nc) in enumerate(chunks):
        ocopy(c).wait()
        if nc == HD:
            proj(done, r0 + nr)
            done = r0 + nr
            continue
        s = _dot(o2[:, c0:c0 + nc], wot_buf[r0:r0 + nr, c0:c0 + nc], _NT)
        acc = s if c0 == 0 else acc + s
        if c0 + nc == HD:
            finish(acc, r0, nr)

    cp = pltpu.make_async_copy(out_buf, o_hbm, sem_o.at[0])
    cp.start()
    cp.wait()


def _kernel(*refs, B, D, F, HKV, SK, W):
    dma = pltpu.SemaphoreType.DMA
    pl.run_scoped(
        functools.partial(_body, *refs, B=B, D=D, F=F, HKV=HKV, SK=SK, W=W),
        dma((5,)), dma((2,)), dma((2,)), dma((2,)), dma((2,)), dma((1,)),
        dma((len(_ROW_SPLIT) + len(_TAIL_COLS),)), dma((1,)))


@jax.jit
def pallas_recurrent_scan__sliding_block_cached__dense_activation_gelu__decode_kernel(
    A_x: jax.Array,
    A_k_cache: jax.Array,
    A_v_cache: jax.Array,
    A_wq: jax.Array,
    A_wo: jax.Array,
    B_x: jax.Array,
    B_w1: jax.Array,
    B_b1: jax.Array,
    B_w2: jax.Array,
    B_b2: jax.Array,
):
    B, SQ, D = A_x.shape
    _, HKV, SK, DH = A_k_cache.shape
    F = B_w1.shape[1]
    W = min(4096, max(256, SK // 4))
    HD = _HQ * _DH
    assert B == 2 and SQ == 1 and DH == _DH and A_wq.shape[1] == HD
    assert _HQ == 2 * HKV and D == 576
    bf = jnp.bfloat16
    npair = B * HKV

    any_spec = pl.BlockSpec(memory_space=pl.ANY)
    out = pl.pallas_call(
        functools.partial(_kernel, B=B, D=D, F=F, HKV=HKV, SK=SK, W=W),
        out_shape=jax.ShapeDtypeStruct((B, D), A_x.dtype),
        in_specs=[any_spec] * 9,
        out_specs=any_spec,
        scratch_shapes=[
            pltpu.VMEM((B, D), bf),
            pltpu.VMEM((F,), bf),
            pltpu.VMEM((D,), bf),
            pltpu.VMEM((D, HD), bf),
            pltpu.VMEM((D, HD), bf),
            pltpu.VMEM((D, F), bf),
            pltpu.VMEM((D, F), bf),
            pltpu.VMEM((npair, W, _DH), bf),
            pltpu.VMEM((npair, W, _DH), bf),
            pltpu.VMEM((8, HD), jnp.float32),
            pltpu.VMEM((8, HD), jnp.float32),
            pltpu.VMEM((8, D), bf),
            pltpu.VMEM((8, F), bf),
            pltpu.VMEM((8, D), jnp.float32),
            pltpu.VMEM((B, D), bf),
            pltpu.SMEM((_NSLOT, _PROWS, HD), bf),
        ],
        compiler_params=pltpu.CompilerParams(vmem_limit_bytes=110 * 1024 * 1024),
    )(A_x.reshape(B, D), A_k_cache, A_v_cache, A_wq, A_wo.T, B_w1, B_b1, B_w2.T, B_b2)
    return out.reshape(B, SQ, D)
```

```python
import functools

import jax
import jax.numpy as jnp
import jax.experimental.pallas as pl
import jax.experimental.pallas.tpu as pltpu

_HQ = 32
_DH = 128
_EPS = 1e-5
_NT = (((1,), (1,)), ((), ()))
_NN = (((1,), (0,)), ((), ()))

_NSLOT = 3
_PROWS = 8
_NPIECE = 37
_W1_AT = 4
_W2_AT = 10
_ROW_SPLIT = (384, 448, 512)
_TAIL_COLS = (2560, 1536)


def _dot(a, b, dims):
    return jax.lax.dot_general(a, b, dims, precision=jax.lax.Precision.DEFAULT,
                               preferred_element_type=jnp.float32)


def _gelu_tanh(x):
    c = 0.7978845608028654
    return 0.5 * x * (1.0 + jnp.tanh(c * (x + 0.044715 * (x * x * x))))


def _wo_chunks(rows, cols):
    chunks = []
    r = _NPIECE * _PROWS
    for e in _ROW_SPLIT:
        chunks.append((r, e - r, 0, cols))
        r = e
    c = 0
    for n in _TAIL_COLS:
        chunks.append((r, rows - r, c, n))
        c += n
    assert c == cols
    return chunks


def _body(x_hbm, k_hbm, v_hbm, wq_hbm, wot_hbm, w1_hbm, b1_hbm, w2t_hbm, b2_hbm, o_hbm,
          x_buf, b1_buf, b2_buf, wq_buf, wot_buf, w1_buf, w2t_buf, k_buf, v_buf,
          q_buf, o_buf, xn_buf, h_buf, g_buf, acc_buf, out_buf, stage,
          sem_first, sem_w, sem_k, sem_v, sem_in, sem_out, sem_c, sem_o,
          *, B, D, F, HKV, SK, W):
    s0 = SK - W
    npair = B * HKV
    HD = _HQ * _DH
    half = D // 2
    NP = _NPIECE
    A1, A2 = _W1_AT, _W2_AT
    side_rows = NP * _PROWS
    chunks = _wo_chunks(D, HD)
    assert NP <= 2 + npair + 4 - 1

    def first(i):
        src, dst = [(wq_hbm.at[pl.ds(0, half)], wq_buf.at[pl.ds(0, half)]),
                    (wq_hbm.at[pl.ds(half, half)], wq_buf.at[pl.ds(half, half)]),
                    (x_hbm, x_buf), (b1_hbm, b1_buf), (b2_hbm, b2_buf)][i]
        return pltpu.make_async_copy(src, dst, sem_first.at[i])

    def wcopy(which, h):
        src, dst = [(w1_hbm, w1_buf), (w2t_hbm, w2t_buf)][which]
        return pltpu.make_async_copy(src.at[pl.ds(h * half, half)],
                                     dst.at[pl.ds(h * half, half)], sem_w.at[h])

    def kcopy(p):
        return pltpu.make_async_copy(
            k_hbm.at[p % B, p // B, pl.ds(s0, W), :], k_buf.at[p], sem_k.at[p % 2])

    def vcopy(p):
        return pltpu.make_async_copy(
            v_hbm.at[p % B, p // B, pl.ds(s0, W), :], v_buf.at[p], sem_v.at[p % 2])

    def ocopy(c):
        r0, nr, c0, nc = chunks[c]
        return pltpu.make_async_copy(
            wot_hbm.at[pl.ds(r0, nr), pl.ds(c0, nc)],
            wot_buf.at[pl.ds(r0, nr), pl.ds(c0, nc)], sem_c.at[c])

    def rows(k):
        if isinstance(k, int):
            return pl.ds(k * _PROWS, _PROWS)
        return pl.ds(pl.multiple_of(k * _PROWS, _PROWS), _PROWS)

    def cin(k):
        return pltpu.make_async_copy(wot_hbm.at[rows(k)], stage.at[k % _NSLOT],
                                     sem_in.at[k % 2])

    def cout(k):
        return pltpu.make_async_copy(stage.at[k % _NSLOT], wot_buf.at[rows(k)],
                                     sem_out.at[0])

    def when(cond):
        if isinstance(cond, bool):
            return (lambda f: f()) if cond else (lambda f: None)
        return pl.when(cond)

    def pinned(cond, fn):
        if isinstance(cond, bool):
            when(cond)(fn)
            return

        def step(i, c):
            fn()
            return c
        jax.lax.fori_loop(0, cond.astype(jnp.int32), step, 0)

    def service(t):
        @when(t < NP)
        def _():
            cin(t).wait()

        if not (isinstance(t, int) and t == 0):
            @when(t <= NP)
            def _():
                cout(t - 1).wait()

        def starts():
            @when(t + 2 < NP)
            def _():
                cin(t + 2).start()
            cout(t).start()

        pinned(t < NP, starts)

    for i in range(5):
        first(i).start()
    cin(0).start()
    cin(1).start()

    def prime(p, c):
        kcopy(p).start()
        vcopy(p).start()
        return c

    jax.lax.fori_loop(0, 2, prime, 0)

    first(0).wait()
    service(0)
    for i in range(1, 5):
        first(i).wait()
    service(1)

    x = x_buf[...].astype(jnp.float32)
    mu = jnp.mean(x, axis=-1, keepdims=True)
    xc = x - mu
    var = jnp.mean(xc * xc, axis=-1, keepdims=True)
    xn = xc * jax.lax.rsqrt(var + _EPS)
    row_d = jax.lax.broadcasted_iota(jnp.int32, (8, D), 0)
    xn8 = jnp.where(row_d % 2 == 0, xn[0:1, :], xn[1:2, :]).astype(jnp.bfloat16)
    xn_buf[...] = xn8
    q_buf[...] = _dot(xn8, wq_buf[...], _NN)

    row = jax.lax.broadcasted_iota(jnp.int32, (8, _DH), 0)
    scale = _DH ** -0.5

    def step(p, c):
        j = p // B
        b = p % B
        off_a = pl.multiple_of(2 * j * _DH, _DH)
        off_b = pl.multiple_of((2 * j + 1) * _DH, _DH)
        tick = (2 + p + (p > A1).astype(jnp.int32) + (p > A1 + 1).astype(jnp.int32)
                + (p > A2).astype(jnp.int32) + (p > A2 + 1).astype(jnp.int32))
        lhs = jnp.where(row < 2, q_buf[:, pl.ds(off_a, _DH)],
                        q_buf[:, pl.ds(off_b, _DH)]).astype(jnp.bfloat16)
        kcopy(p).wait()
        vcopy(p).wait()

        @pl.when(p + 2 < npair)
        def _():
            kcopy(p + 2).start()
            vcopy(p + 2).start()

        @pl.when(p == npair - 2)
        def _():
            ocopy(0).start()
            ocopy(1).start()

        service(tick)

        @pl.when(p == npair - 1)
        def _():
            for c in range(2, len(chunks)):
                ocopy(c).start()

        s = _dot(lhs, k_buf[p], _NT)
        m = jnp.max(s, axis=-1, keepdims=True)
        e = jnp.exp((s - m) * scale)
        l = jnp.sum(e, axis=-1, keepdims=True)
        o = _dot(e.astype(jnp.bfloat16), v_buf[p], _NN) / l
        o_sh = pltpu.roll(o, 6, 0)

        @pl.when(b == 0)
        def _():
            o_buf[:, pl.ds(off_a, _DH)] = jnp.where(row == 0, o, 0.0)
            o_buf[:, pl.ds(off_b, _DH)] = jnp.where(row == 0, o_sh, 0.0)

        @pl.when(b == 1)
        def _():
            o_buf[:, pl.ds(off_a, _DH)] = jnp.where(row == 1, o, o_buf[:, pl.ds(off_a, _DH)])
            o_buf[:, pl.ds(off_b, _DH)] = jnp.where(row == 1, o_sh, o_buf[:, pl.ds(off_b, _DH)])

        for which, at in ((0, A1), (1, A2)):
            for h in range(2):
                @pl.when(p == at - 2 + h)
                def _():
                    wcopy(which, h).start()

        @pl.when(p == A1)
        def _():
            wcopy(0, 0).wait()
            service(2 + A1 + 1)

        @pl.when(p == A1 + 1)
        def _():
            wcopy(0, 1).wait()
            service(2 + A1 + 3)
            h = _dot(xn_buf[...], w1_buf[...], _NN)
            h = _gelu_tanh(h + b1_buf[...].astype(jnp.float32).reshape(1, F))
            h_buf[...] = h.astype(jnp.bfloat16)

        @pl.when(p == A2)
        def _():
            wcopy(1, 0).wait()
            service(2 + A2 + 3)

        @pl.when(p == A2 + 1)
        def _():
            wcopy(1, 1).wait()
            service(2 + A2 + 5)
            y = _dot(h_buf[...], w2t_buf[...], _NT)
            y = y + b2_buf[...].astype(jnp.float32).reshape(1, D)
            g_buf[...] = y * jax.nn.sigmoid(y)

        return c

    jax.lax.fori_loop(0, npair, step, 0)

    o2 = o_buf[...].astype(jnp.bfloat16)
    xf = x_buf[...].astype(jnp.float32)

    def finish(s, r0, nr):
        out_buf[:, r0:r0 + nr] = (xf[:, r0:r0 + nr]
                                  + s[0:2, :] * g_buf[0:2, r0:r0 + nr]).astype(out_buf.dtype)

    def proj(r0, r1):
        finish(_dot(o2, wot_buf[r0:r1, :], _NT), r0, r1 - r0)

    done = 0
    while done + 128 <= side_rows:
        proj(done, done + 128)
        done += 128
    for c, (r0, nr, c0, nc) in enumerate(chunks):
        ocopy(c).wait()
        if nc == HD:
            proj(done, r0 + nr)
            done = r0 + nr
            continue
        s = _dot(o2[:, c0:c0 + nc], wot_buf[r0:r0 + nr, c0:c0 + nc], _NT)
        if c0 > 0:
            s = s + acc_buf[:, 0:nr]
        if c0 + nc < HD:
            acc_buf[:, 0:nr] = s
        else:
            finish(s, r0, nr)

    cp = pltpu.make_async_copy(out_buf, o_hbm, sem_o.at[0])
    cp.start()
    cp.wait()


def _kernel(*refs, B, D, F, HKV, SK, W):
    dma = pltpu.SemaphoreType.DMA
    pl.run_scoped(
        functools.partial(_body, *refs, B=B, D=D, F=F, HKV=HKV, SK=SK, W=W),
        dma((5,)), dma((2,)), dma((2,)), dma((2,)), dma((2,)), dma((1,)),
        dma((len(_ROW_SPLIT) + len(_TAIL_COLS),)), dma((1,)))


@jax.jit
def pallas_recurrent_scan__sliding_block_cached__dense_activation_gelu__decode_kernel(
    A_x: jax.Array,
    A_k_cache: jax.Array,
    A_v_cache: jax.Array,
    A_wq: jax.Array,
    A_wo: jax.Array,
    B_x: jax.Array,
    B_w1: jax.Array,
    B_b1: jax.Array,
    B_w2: jax.Array,
    B_b2: jax.Array,
):
    B, SQ, D = A_x.shape
    _, HKV, SK, DH = A_k_cache.shape
    F = B_w1.shape[1]
    W = min(4096, max(256, SK // 4))
    HD = _HQ * _DH
    assert B == 2 and SQ == 1 and DH == _DH and A_wq.shape[1] == HD
    assert _HQ == 2 * HKV and D == 576
    bf = jnp.bfloat16
    npair = B * HKV

    any_spec = pl.BlockSpec(memory_space=pl.ANY)
    out = pl.pallas_call(
        functools.partial(_kernel, B=B, D=D, F=F, HKV=HKV, SK=SK, W=W),
        out_shape=jax.ShapeDtypeStruct((B, D), A_x.dtype),
        in_specs=[any_spec] * 9,
        out_specs=any_spec,
        scratch_shapes=[
            pltpu.VMEM((B, D), bf),
            pltpu.VMEM((F,), bf),
            pltpu.VMEM((D,), bf),
            pltpu.VMEM((D, HD), bf),
            pltpu.VMEM((D, HD), bf),
            pltpu.VMEM((D, F), bf),
            pltpu.VMEM((D, F), bf),
            pltpu.VMEM((npair, W, _DH), bf),
            pltpu.VMEM((npair, W, _DH), bf),
            pltpu.VMEM((8, HD), jnp.float32),
            pltpu.VMEM((8, HD), jnp.float32),
            pltpu.VMEM((8, D), bf),
            pltpu.VMEM((8, F), bf),
            pltpu.VMEM((8, D), jnp.float32),
            pltpu.VMEM((8, 128), jnp.float32),
            pltpu.VMEM((B, D), bf),
            pltpu.SMEM((_NSLOT, _PROWS, HD), bf),
        ],
        compiler_params=pltpu.CompilerParams(vmem_limit_bytes=110 * 1024 * 1024),
    )(A_x.reshape(B, D), A_k_cache, A_v_cache, A_wq, A_wo.T, B_w1, B_b1, B_w2.T, B_b2)
    return out.reshape(B, SQ, D)
```
